```python
import os as _os
_os.environ.setdefault('JAX_PLATFORMS', 'cpu')
import jax
import jax.numpy as jnp

def _softmax(x, axis=-1):
    return jax.nn.softmax(x, axis=axis)

def _gelu(x):
    return jax.nn.gelu(x, approximate=True)

def _silu(x):
    return jax.nn.silu(x)

def _sigmoid(x):
    return jax.nn.sigmoid(x)

def _layernorm(x, axis=-1, eps=1e-05):
    m = jnp.mean(x, axis=axis, keepdims=True)
    v = jnp.var(x, axis=axis, keepdims=True)
    return (x - m) / jnp.sqrt(v + eps)

def _scatter_add(tgt, idx, src, axis=0):
    return tgt.at[idx].add(src)

def _segment_sum(src, seg, n):
    return jax.ops.segment_sum(src, seg, n)

class _Rng:

    def __init__(self, key):
        self._k = key

    def _next(self):
        self._k, sub = jax.random.split(self._k)
        return sub

    def normal(self, shape):
        return jax.random.normal(self._next(), shape, dtype=jnp.bfloat16)

    def randint(self, lo, hi, shape):
        return jax.random.randint(self._next(), shape, lo, hi, dtype=jnp.int32)

    def uniform(self, shape, lo=0.0, hi=1.0):
        return jax.random.uniform(self._next(), shape, jnp.bfloat16, lo, hi)

    def permutation(self, n):
        return jax.random.permutation(self._next(), n)
kernel_name = 'adaLN_cond__mha_block__dense_activation_squared_relu__prompt'

def setup_inputs():
    _rng = _Rng(jax.random.key(int.from_bytes(__import__("os").urandom(4), "little")))
    _w = lambda a: (lambda t: t.astype(jnp.bfloat16) if jnp.issubdtype(t.dtype, jnp.floating) else t)(jnp.asarray(a))

    def _A_setup():
        B, S, D, H = (1, 2048, 512, 32)
        return {'x': _w((lambda *s: _rng.normal(s) * 0.05)(B, S, D)), 'wqkv': _w((lambda *s: _rng.normal(s) * 0.1)(D, 3 * D)), 'wo': _w((lambda *s: _rng.normal(s) * 0.05)(D, D))}
    _A_in = _A_setup()

    def _B_setup():
        B, S, D, F = (1, 2048, 512, 1792)
        return {'x': _w((lambda *s: _rng.normal(s) * 0.05)(B, S, D)), 'w1': _w((lambda *s: _rng.normal(s) * 0.05)(D, F)), 'b1': _w((lambda *s: _rng.normal(s) * 0.05)(F)), 'w2': _w((lambda *s: _rng.normal(s) * 0.05)(F, D)), 'b2': _w((lambda *s: _rng.normal(s) * 0.05)(D))}
    _B_in = _B_setup()
    return {'A_x': _A_in['x'], 'A_wqkv': _A_in['wqkv'], 'A_wo': _A_in['wo'], 'B_x': _B_in['x'], 'B_w1': _B_in['w1'], 'B_b1': _B_in['b1'], 'B_w2': _B_in['w2'], 'B_b2': _B_in['b2'], 'c': _w((lambda *s: _rng.normal(s) * 0.05)(1, 512) * 8.0), 'w_mod': _w((lambda *s: _rng.normal(s) * 0.05)(512, 6 * 512) * 512 ** (-0.5) * 8.0)}

def reference(A_x, A_wqkv, A_wo, B_x, B_w1, B_b1, B_w2, B_b2, c, w_mod):

    def _A_ref(x, wqkv, wo):
        B, S, D = x.shape
        H = 32
        Dh = D // H
        qkv = (lambda x, *d: x.transpose(*d))((x @ wqkv).reshape(B, S, 3, H, Dh), 2, 0, 3, 1, 4)
        q, k, v = (qkv[0], qkv[1], qkv[2])
        scores = jnp.einsum('bhqd,bhkd->bhqk', q, k) * Dh ** (-0.5)
        p = _softmax(scores, axis=-1)
        o = jnp.einsum('bhqk,bhkd->bhqd', p, v)
        return (lambda x, *d: x.transpose(*d))(o, 0, 2, 1, 3).reshape(B, S, D) @ wo

    def _B_ref(x, w1, b1, w2, b2):
        h = jnp.einsum('bsd,df->bsf', x, w1) + b1
        zero = jnp.zeros_like(h)
        r = jnp.where(h > zero, h, zero)
        h = r * r
        out = jnp.einsum('bsf,fd->bsd', h, w2) + b2
        return out
    x = A_x
    mod = (_silu(c) @ w_mod).reshape(c.shape[0], 6, 1, -1)
    sa, ca, ga, sb, cb, gb = (mod[:, 0].copy(), mod[:, 1].copy(), mod[:, 2].copy(), mod[:, 3].copy(), mod[:, 4].copy(), mod[:, 5].copy())
    h = _layernorm(x, axis=-1) * (1 + ca) + sa
    x = x + ga * _A_ref(h, A_wqkv, A_wo)
    h = _layernorm(x, axis=-1) * (1 + cb) + sb
    x = x + gb * _B_ref(h, B_w1, B_b1, B_w2, B_b2)
    return x
```

```python
import math
import jax
import jax.numpy as jnp
import jax.experimental.pallas as pl
import jax.experimental.pallas.tpu as pltpu

S = 2048
D = 512
H = 32
DH = 16
F = 1792
TQ = 256
NQ = S // TQ
CK = 128
NC = S // CK
LAG = 4
DEP = 2
NP = 5
EPS = 1e-5
LOG2E = math.log2(math.e)
f32 = jnp.float32
bf16 = jnp.bfloat16


def _ln(xf):
    mu = jnp.mean(xf, axis=-1, keepdims=True)
    xc = xf - mu
    var = jnp.mean(xc * xc, axis=-1, keepdims=True)
    return xc * jax.lax.rsqrt(var + EPS)


def _kernel(x_hbm, wqkv_hbm, wo_hbm, w1_hbm, b1_ref, w2_hbm, b2_ref, c_ref, wmod_hbm,
            o_ref,
            x_v, wqkv_v, wo_v, w1_v, w2_v, wmod_v, sems,
            mod_sc, k_sc, qt_sc, vt_sc, ot_sc, sa_sc, sb_sc, m0_sc):
    i = pl.program_id(0)
    row128 = jax.lax.broadcasted_iota(jnp.int32, (128, TQ), 0)

    def cp_wmod_a():
        return pltpu.make_async_copy(wmod_hbm.at[:, pl.ds(0, 2 * D)], wmod_v.at[:, pl.ds(0, 2 * D)], sems.at[0])

    def cp_wmod_b():
        return pltpu.make_async_copy(wmod_hbm.at[:, pl.ds(2 * D, 4 * D)], wmod_v.at[:, pl.ds(2 * D, 4 * D)], sems.at[1])

    def cp_wqkv():
        return pltpu.make_async_copy(wqkv_hbm, wqkv_v, sems.at[2])

    def cp_wo():
        return pltpu.make_async_copy(wo_hbm, wo_v, sems.at[3])

    def cp_w1():
        return pltpu.make_async_copy(w1_hbm, w1_v, sems.at[4])

    def cp_w2():
        return pltpu.make_async_copy(w2_hbm, w2_v, sems.at[5])

    def cp_x(r):
        lo, n = (0, TQ) if r == 0 else (TQ, S - TQ)
        return pltpu.make_async_copy(x_hbm.at[pl.ds(lo, n), :], x_v.at[pl.ds(lo, n), :], sems.at[6 + r])

    def qmask(blk, h):
        g = h // 8
        hh = h % 8
        qg = qt_sc[blk, pl.ds(pl.multiple_of(g * 128, 128), 128), :]
        return g, jnp.where((row128 >= hh * 16) & (row128 < hh * 16 + 16), qg, jnp.zeros_like(qg))

    def qk_chunk(g, qm, c, buf, mx):
        s = jnp.dot(k_sc[g, c * CK:(c + 1) * CK, :], qm, preferred_element_type=f32)
        buf[c * CK:(c + 1) * CK, :] = s
        cm = jnp.max(s.reshape(CK // 8, 8, TQ), axis=0)
        return cm if mx is None else jnp.maximum(mx, cm)

    toks = []

    def pv_chunk(h, c, buf, m, acc):
        tok = toks[-DEP] if len(toks) >= DEP else None
        m8 = jnp.broadcast_to(m, (8, TQ)) if tok is None else m + (tok - tok)
        p = jnp.exp2(buf[c * CK:(c + 1) * CK, :].reshape(CK // 8, 8, TQ) - m8[None])
        cl = jnp.sum(p, axis=0)
        toks.append(cl)
        o = jnp.dot(vt_sc[h, :, c * CK:(c + 1) * CK], p.reshape(CK, TQ).astype(bf16), preferred_element_type=f32)
        if acc is None:
            return cl, o
        return acc[0] + cl, acc[1] + o

    def finalize(h, acc):
        l = jnp.sum(acc[0], axis=0, keepdims=True)
        ot_sc[pl.ds(pl.multiple_of(h * 16, 16), 16), :] = acc[1] / l

    def half(blk_q, h_q, wbuf, rbuf, tail, head):
        g, qm = qmask(blk_q, h_q)
        mx = None
        acc = None
        for c in range(NC):
            mx = qk_chunk(g, qm, c, wbuf, mx)
            if c < LAG:
                if tail is not None:
                    tail = (tail[0], tail[1], pv_chunk(tail[0], NC - LAG + c, wbuf, tail[1], tail[2]))
                    if c == LAG - 1:
                        finalize(tail[0], tail[2])
            elif head is not None:
                acc = pv_chunk(head[0], c - LAG, rbuf, head[1], acc)
        return jnp.max(mx, axis=0, keepdims=True), acc

    @pl.when(i == 0)
    def _prologue():
        cp_wmod_a().start()
        cp_x(0).start()
        cp_wqkv().start()
        cp_x(1).start()
        cp_wmod_b().start()
        cp_wo().start()
        cp_w1().start()
        cp_w2().start()
        c = jnp.broadcast_to(c_ref[...].astype(f32), (8, D))
        sc = (c * jax.nn.sigmoid(c)).astype(bf16)
        cp_wmod_a().wait()
        mod_sc[:, 0:2 * D] = jnp.dot(sc, wmod_v[:, 0:2 * D], preferred_element_type=f32)
        sa = mod_sc[0:1, 0:D]
        ca = mod_sc[0:1, D:2 * D]
        for r in range(NQ):
            if r < 2:
                cp_x(r).wait()
            if r == 0:
                cp_wqkv().wait()
            xf = x_v[r * TQ:(r + 1) * TQ, :].astype(f32)
            h = _ln(xf) * (1.0 + ca) + sa
            qkv = jnp.dot(h.astype(bf16), wqkv_v[...], preferred_element_type=f32)
            kk = qkv[:, D:2 * D].astype(bf16)
            for g in range(4):
                k_sc[g, r * TQ:(r + 1) * TQ, :] = kk[:, g * 128:(g + 1) * 128]
            qt_sc[r] = (qkv[:, 0:D] * (DH ** -0.5 * LOG2E)).T.astype(bf16)
            vt = qkv[:, 2 * D:3 * D].T.astype(bf16)
            vt_sc[:, :, r * TQ:(r + 1) * TQ] = vt.reshape(H, DH, TQ)
        cp_wmod_b().wait()
        mod_sc[:, 2 * D:6 * D] = jnp.dot(sc, wmod_v[:, 2 * D:6 * D], preferred_element_type=f32)
        m, _ = half(0, 0, sa_sc, None, None, None)
        m0_sc[...] = jnp.broadcast_to(m, (8, TQ))
        cp_wo().wait()
        cp_w1().wait()
        cp_w2().wait()

    toks.clear()
    m_0 = m0_sc[0:1, :]
    m_1, acc0 = half(i, 1, sb_sc, sa_sc, None, (0, m_0))

    NPAIR = H // 2 - 1

    def pair(h, carry):
        m_p, la_p, oa_p, m_c = carry
        m_n, acc_c = half(i, h, sa_sc, sb_sc, (h - 2, m_p, (la_p, oa_p)), (h - 1, m_c))
        m_n2, acc_n = half(i, h + 1, sb_sc, sa_sc, (h - 1, m_c, acc_c), (h, m_n))
        return m_n, acc_n[0], acc_n[1], m_n2

    carry = (m_0, acc0[0], acc0[1], m_1)
    rem = NPAIR % NP
    for r in range(rem):
        carry = pair(2 * r + 2, carry)

    def body(j, carry):
        toks.clear()
        for r in range(NP):
            carry = pair(2 * (rem + j * NP + r) + 2, carry)
        return carry

    m_p, la_p, oa_p, m_c = jax.lax.fori_loop(0, NPAIR // NP, body, carry)
    toks.clear()
    nxt = jnp.minimum(i + 1, NQ - 1)
    m_n, acc_c = half(nxt, 0, sa_sc, sb_sc, (H - 2, m_p, (la_p, oa_p)), (H - 1, m_c))
    m0_sc[...] = jnp.broadcast_to(m_n, (8, TQ))
    for c in range(NC - LAG, NC):
        acc_c = pv_chunk(H - 1, c, sb_sc, m_c, acc_c)
    finalize(H - 1, acc_c)

    ga = mod_sc[0:1, 2 * D:3 * D]
    sb = mod_sc[0:1, 3 * D:4 * D]
    cb = mod_sc[0:1, 4 * D:5 * D]
    gb = mod_sc[0:1, 5 * D:6 * D]
    o_att = ot_sc[...].T.astype(bf16)
    att = jnp.dot(o_att, wo_v[...], preferred_element_type=f32)
    rows = pl.ds(pl.multiple_of(i * TQ, TQ), TQ)
    x1 = x_v[rows, :].astype(f32) + ga * att
    h2 = _ln(x1) * (1.0 + cb) + sb
    u = jnp.dot(h2.astype(bf16), w1_v[...], preferred_element_type=f32) + b1_ref[...].astype(f32)
    u = jnp.maximum(u, 0.0)
    u = u * u
    y = jnp.dot(u.astype(bf16), w2_v[...], preferred_element_type=f32) + b2_ref[...].astype(f32)
    o_ref[...] = (x1 + gb * y).astype(o_ref.dtype)


@jax.jit
def pallas_adaLN_cond__mha_block__dense_activation_squared_relu__prompt_kernel(
    A_x, A_wqkv, A_wo, B_x, B_w1, B_b1, B_w2, B_b2, c, w_mod):
    del B_x
    x = A_x.reshape(S, D)
    full = lambda shape: pl.BlockSpec(shape, lambda i: (0,) * len(shape))
    hbm = pl.BlockSpec(memory_space=pl.ANY)
    out = pl.pallas_call(
        _kernel,
        grid=(NQ,),
        in_specs=[hbm, hbm, hbm, hbm, full((1, F)), hbm, full((1, D)), full((1, D)), hbm],
        out_specs=pl.BlockSpec((TQ, D), lambda i: (i, 0)),
        out_shape=jax.ShapeDtypeStruct((S, D), bf16),
        scratch_shapes=[
            pltpu.VMEM((S, D), bf16),
            pltpu.VMEM((D, 3 * D), bf16),
            pltpu.VMEM((D, D), bf16),
            pltpu.VMEM((D, F), bf16),
            pltpu.VMEM((F, D), bf16),
            pltpu.VMEM((D, 6 * D), bf16),
            pltpu.SemaphoreType.DMA((8,)),
            pltpu.VMEM((8, 6 * D), f32),
            pltpu.VMEM((4, S, 128), bf16),
            pltpu.VMEM((NQ, D, TQ), bf16),
            pltpu.VMEM((H, DH, S), bf16),
            pltpu.VMEM((D, TQ), f32),
            pltpu.VMEM((S, TQ), f32),
            pltpu.VMEM((S, TQ), f32),
            pltpu.VMEM((8, TQ), f32),
        ],
        compiler_params=pltpu.CompilerParams(
            dimension_semantics=("arbitrary",),
            vmem_limit_bytes=100 * 1024 * 1024,
        ),
    )(x, A_wqkv, A_wo, B_w1, B_b1.reshape(1, F), B_w2, B_b2.reshape(1, D), c, w_mod)
    return out.reshape(1, S, D)
```

```python
import math
import jax
import jax.numpy as jnp
import jax.experimental.pallas as pl
import jax.experimental.pallas.tpu as pltpu

S = 2048
D = 512
H = 32
DH = 16
F = 1792
TQ = 256
NQ = S // TQ
CK = 128
NC = S // CK
LAG = 3
DEP = 1
NP = 5
EPS = 1e-5
LOG2E = math.log2(math.e)
f32 = jnp.float32
bf16 = jnp.bfloat16


def _ln(xf):
    mu = jnp.mean(xf, axis=-1, keepdims=True)
    xc = xf - mu
    var = jnp.mean(xc * xc, axis=-1, keepdims=True)
    return xc * jax.lax.rsqrt(var + EPS)


def _tree(x, op):
    parts = [x[j] for j in range(x.shape[0])]
    while len(parts) > 1:
        parts = [op(parts[j], parts[j + 1]) for j in range(0, len(parts) - 1, 2)] + (
            [parts[-1]] if len(parts) % 2 else [])
    return parts[0]


def _kernel(x_hbm, wqkv_hbm, wo_hbm, w1_hbm, b1_ref, w2_hbm, b2_ref, c_ref, wmod_hbm,
            o_ref,
            x_v, wqkv_v, wo_v, w1_v, w2_v, wmod_v, sems,
            mod_sc, k_sc, qt_sc, vt_sc, ot_sc, sa_sc, sb_sc, m0_sc):
    i = pl.program_id(0)
    row128 = jax.lax.broadcasted_iota(jnp.int32, (128, TQ), 0)

    def cp_wmod_a():
        return pltpu.make_async_copy(wmod_hbm.at[:, pl.ds(0, 2 * D)], wmod_v.at[:, pl.ds(0, 2 * D)], sems.at[0])

    def cp_wmod_b():
        return pltpu.make_async_copy(wmod_hbm.at[:, pl.ds(2 * D, 4 * D)], wmod_v.at[:, pl.ds(2 * D, 4 * D)], sems.at[1])

    def cp_wqkv():
        return pltpu.make_async_copy(wqkv_hbm, wqkv_v, sems.at[2])

    def cp_wo():
        return pltpu.make_async_copy(wo_hbm, wo_v, sems.at[3])

    def cp_w1():
        return pltpu.make_async_copy(w1_hbm, w1_v, sems.at[4])

    def cp_w2():
        return pltpu.make_async_copy(w2_hbm, w2_v, sems.at[5])

    def cp_x(r):
        lo, n = (0, TQ) if r == 0 else (TQ, S - TQ)
        return pltpu.make_async_copy(x_hbm.at[pl.ds(lo, n), :], x_v.at[pl.ds(lo, n), :], sems.at[6 + r])

    def qmask(blk, h):
        g = h // 8
        hh = h % 8
        qg = qt_sc[blk, pl.ds(pl.multiple_of(g * 128, 128), 128), :]
        return g, jnp.where((row128 >= hh * 16) & (row128 < hh * 16 + 16), qg, jnp.zeros_like(qg))

    def qk_chunk(g, qm, c, buf, mx):
        s = jnp.dot(k_sc[g, c * CK:(c + 1) * CK, :], qm, preferred_element_type=f32)
        buf[c * CK:(c + 1) * CK, :] = s
        cm = _tree(s.reshape(CK // 8, 8, TQ), jnp.maximum) if 1 else jnp.max(s.reshape(CK // 8, 8, TQ), axis=0)
        return cm if mx is None else jnp.maximum(mx, cm)

    toks = []

    def pv_chunk(h, c, buf, m, acc):
        tok = toks[-DEP] if len(toks) >= DEP else None
        m8 = jnp.broadcast_to(m, (8, TQ)) if tok is None else m + (tok - tok)
        p = jnp.exp2(buf[c * CK:(c + 1) * CK, :].reshape(CK // 8, 8, TQ) - m8[None])
        cl = _tree(p, jnp.add) if 1 else jnp.sum(p, axis=0)
        toks.append(cl)
        o = jnp.dot(vt_sc[h, :, c * CK:(c + 1) * CK], p.reshape(CK, TQ).astype(bf16), preferred_element_type=f32)
        if acc is None:
            return cl, o
        return acc[0] + cl, acc[1] + o

    def finalize(h, acc):
        l = jnp.sum(acc[0], axis=0, keepdims=True)
        ot_sc[pl.ds(pl.multiple_of(h * 16, 16), 16), :] = acc[1] / l

    def half(blk_q, h_q, wbuf, rbuf, tail, head):
        g, qm = qmask(blk_q, h_q)
        mx = None
        acc = None
        for c in range(NC):
            mx = qk_chunk(g, qm, c, wbuf, mx)
            if c < LAG:
                if tail is not None:
                    tail = (tail[0], tail[1], pv_chunk(tail[0], NC - LAG + c, wbuf, tail[1], tail[2]))
                    if c == LAG - 1:
                        finalize(tail[0], tail[2])
            elif head is not None:
                acc = pv_chunk(head[0], c - LAG, rbuf, head[1], acc)
        return jnp.max(mx, axis=0, keepdims=True), acc

    @pl.when(i == 0)
    def _prologue():
        cp_wmod_a().start()
        cp_x(0).start()
        cp_wqkv().start()
        cp_x(1).start()
        cp_wmod_b().start()
        cp_wo().start()
        cp_w1().start()
        cp_w2().start()
        c = jnp.broadcast_to(c_ref[...].astype(f32), (8, D))
        sc = (c * jax.nn.sigmoid(c)).astype(bf16)
        cp_wmod_a().wait()
        mod_sc[:, 0:2 * D] = jnp.dot(sc, wmod_v[:, 0:2 * D], preferred_element_type=f32)
        sa = mod_sc[0:1, 0:D]
        ca = mod_sc[0:1, D:2 * D]
        for r in range(NQ):
            if r < 2:
                cp_x(r).wait()
            if r == 0:
                cp_wqkv().wait()
            xf = x_v[r * TQ:(r + 1) * TQ, :].astype(f32)
            h = _ln(xf) * (1.0 + ca) + sa
            qkv = jnp.dot(h.astype(bf16), wqkv_v[...], preferred_element_type=f32)
            kk = qkv[:, D:2 * D].astype(bf16)
            for g in range(4):
                k_sc[g, r * TQ:(r + 1) * TQ, :] = kk[:, g * 128:(g + 1) * 128]
            qt_sc[r] = (qkv[:, 0:D] * (DH ** -0.5 * LOG2E)).T.astype(bf16)
            vt = qkv[:, 2 * D:3 * D].T.astype(bf16)
            vt_sc[:, :, r * TQ:(r + 1) * TQ] = vt.reshape(H, DH, TQ)
        cp_wmod_b().wait()
        mod_sc[:, 2 * D:6 * D] = jnp.dot(sc, wmod_v[:, 2 * D:6 * D], preferred_element_type=f32)
        m, _ = half(0, 0, sa_sc, None, None, None)
        m0_sc[...] = jnp.broadcast_to(m, (8, TQ))
        cp_wo().wait()
        cp_w1().wait()
        cp_w2().wait()

    toks.clear()
    m_0 = m0_sc[0:1, :]
    m_1, acc0 = half(i, 1, sb_sc, sa_sc, None, (0, m_0))

    NPAIR = H // 2 - 1

    def pair(h, carry):
        m_p, la_p, oa_p, m_c = carry
        m_n, acc_c = half(i, h, sa_sc, sb_sc, (h - 2, m_p, (la_p, oa_p)), (h - 1, m_c))
        m_n2, acc_n = half(i, h + 1, sb_sc, sa_sc, (h - 1, m_c, acc_c), (h, m_n))
        return m_n, acc_n[0], acc_n[1], m_n2

    carry = (m_0, acc0[0], acc0[1], m_1)
    rem = NPAIR % NP
    for r in range(rem):
        carry = pair(2 * r + 2, carry)

    def body(j, carry):
        toks.clear()
        for r in range(NP):
            carry = pair(2 * (rem + j * NP + r) + 2, carry)
        return carry

    m_p, la_p, oa_p, m_c = jax.lax.fori_loop(0, NPAIR // NP, body, carry)
    toks.clear()
    nxt = jnp.minimum(i + 1, NQ - 1)
    m_n, acc_c = half(nxt, 0, sa_sc, sb_sc, (H - 2, m_p, (la_p, oa_p)), (H - 1, m_c))
    m0_sc[...] = jnp.broadcast_to(m_n, (8, TQ))
    for c in range(NC - LAG, NC):
        acc_c = pv_chunk(H - 1, c, sb_sc, m_c, acc_c)
    finalize(H - 1, acc_c)

    ga = mod_sc[0:1, 2 * D:3 * D]
    sb = mod_sc[0:1, 3 * D:4 * D]
    cb = mod_sc[0:1, 4 * D:5 * D]
    gb = mod_sc[0:1, 5 * D:6 * D]
    RS = 128
    nr = TQ // RS
    b1 = b1_ref[...].astype(f32).reshape(1, F)
    b2 = b2_ref[...].astype(f32).reshape(1, D)
    x1s = []
    for r in range(nr):
        o_att = ot_sc[:, r * RS:(r + 1) * RS].T.astype(bf16)
        att = jnp.dot(o_att, wo_v[...], preferred_element_type=f32)
        rows = pl.ds(pl.multiple_of(i * TQ + r * RS, RS), RS)
        x1s.append(x_v[rows, :].astype(f32) + ga * att)
    us = []
    for r in range(nr):
        h2 = _ln(x1s[r]) * (1.0 + cb) + sb
        u = jnp.dot(h2.astype(bf16), w1_v[...], preferred_element_type=f32) + b1
        u = jnp.maximum(u, 0.0)
        us.append((u * u).astype(bf16))
    for r in range(nr):
        y = jnp.dot(us[r], w2_v[...], preferred_element_type=f32) + b2
        o_ref[r * RS:(r + 1) * RS, :] = (x1s[r] + gb * y).astype(o_ref.dtype)


@jax.jit
def pallas_adaLN_cond__mha_block__dense_activation_squared_relu__prompt_kernel(
    A_x, A_wqkv, A_wo, B_x, B_w1, B_b1, B_w2, B_b2, c, w_mod):
    del B_x
    x = A_x.reshape(S, D)
    full = lambda shape: pl.BlockSpec(shape, lambda i: (0,) * len(shape))
    hbm = pl.BlockSpec(memory_space=pl.ANY)
    out = pl.pallas_call(
        _kernel,
        grid=(NQ,),
        in_specs=[hbm, hbm, hbm, hbm, full((F,)), hbm, full((D,)), full((1, D)), hbm],
        out_specs=pl.BlockSpec((TQ, D), lambda i: (i, 0)),
        out_shape=jax.ShapeDtypeStruct((S, D), bf16),
        scratch_shapes=[
            pltpu.VMEM((S, D), bf16),
            pltpu.VMEM((D, 3 * D), bf16),
            pltpu.VMEM((D, D), bf16),
            pltpu.VMEM((D, F), bf16),
            pltpu.VMEM((F, D), bf16),
            pltpu.VMEM((D, 6 * D), bf16),
            pltpu.SemaphoreType.DMA((8,)),
            pltpu.VMEM((8, 6 * D), f32),
            pltpu.VMEM((4, S, 128), bf16),
            pltpu.VMEM((NQ, D, TQ), bf16),
            pltpu.VMEM((H, DH, S), bf16),
            pltpu.VMEM((D, TQ), f32),
            pltpu.VMEM((S, TQ), f32),
            pltpu.VMEM((S, TQ), f32),
            pltpu.VMEM((8, TQ), f32),
        ],
        compiler_params=pltpu.CompilerParams(
            dimension_semantics=("arbitrary",),
            vmem_limit_bytes=100 * 1024 * 1024,
        ),
    )(x, A_wqkv, A_wo, B_w1, B_b1, B_w2, B_b2, c, w_mod)
    return out.reshape(1, S, D)
```

```python
import math
import jax
import jax.numpy as jnp
import jax.experimental.pallas as pl
import jax.experimental.pallas.tpu as pltpu

S = 2048
D = 512
H = 32
DH = 16
F = 1792
TQ = 256
NQ = S // TQ
CK = 128
NC = S // CK
LAG = 3
DEP = 1
NP = 5
EPS = 1e-5
LOG2E = math.log2(math.e)
f32 = jnp.float32
bf16 = jnp.bfloat16


def _ln(xf):
    mu = jnp.mean(xf, axis=-1, keepdims=True)
    xc = xf - mu
    var = jnp.mean(xc * xc, axis=-1, keepdims=True)
    return xc * jax.lax.rsqrt(var + EPS)


def _tree(x, op):
    parts = [x[j] for j in range(x.shape[0])]
    while len(parts) > 1:
        parts = [op(parts[j], parts[j + 1]) for j in range(0, len(parts) - 1, 2)] + (
            [parts[-1]] if len(parts) % 2 else [])
    return parts[0]


def _kernel(x_hbm, wqkv_hbm, wo_hbm, w1_hbm, b1_ref, w2_hbm, b2_ref, c_ref, wmod_hbm,
            o_ref,
            x_v, wqkv_v, wo_v, w1_v, w2_v, wmod_v, sems,
            mod_sc, k_sc, qt_sc, vt_sc, ot_sc, sa_sc, sb_sc, m0_sc):
    i = pl.program_id(0)
    row128 = jax.lax.broadcasted_iota(jnp.int32, (128, TQ), 0)

    def cp_wmod_a():
        return pltpu.make_async_copy(wmod_hbm.at[:, pl.ds(0, 2 * D)], wmod_v.at[:, pl.ds(0, 2 * D)], sems.at[0])

    def cp_wmod_b():
        return pltpu.make_async_copy(wmod_hbm.at[:, pl.ds(2 * D, 4 * D)], wmod_v.at[:, pl.ds(2 * D, 4 * D)], sems.at[1])

    def cp_wqkv():
        return pltpu.make_async_copy(wqkv_hbm, wqkv_v, sems.at[2])

    def cp_wo():
        return pltpu.make_async_copy(wo_hbm, wo_v, sems.at[3])

    def cp_w1():
        return pltpu.make_async_copy(w1_hbm, w1_v, sems.at[4])

    def cp_w2():
        return pltpu.make_async_copy(w2_hbm, w2_v, sems.at[5])

    def cp_x(r):
        lo, n = (0, TQ) if r == 0 else (TQ, S - TQ)
        return pltpu.make_async_copy(x_hbm.at[pl.ds(lo, n), :], x_v.at[pl.ds(lo, n), :], sems.at[6 + r])

    def qmask(blk, h):
        g = h // 8
        hh = h % 8
        qg = qt_sc[blk, pl.ds(pl.multiple_of(g * 128, 128), 128), :]
        return g, jnp.where((row128 >= hh * 16) & (row128 < hh * 16 + 16), qg, jnp.zeros_like(qg))

    def qk_chunk(g, qm, c, buf, mx):
        s = jnp.dot(k_sc[g, c * CK:(c + 1) * CK, :], qm, preferred_element_type=f32)
        buf[c * CK:(c + 1) * CK, :] = s
        cm = _tree(s.reshape(CK // 8, 8, TQ), jnp.maximum) if 1 else jnp.max(s.reshape(CK // 8, 8, TQ), axis=0)
        return cm if mx is None else jnp.maximum(mx, cm)

    toks = []

    def pv_chunk(h, c, buf, m, acc):
        tok = toks[-DEP] if len(toks) >= DEP else None
        m8 = jnp.broadcast_to(m, (8, TQ)) if tok is None else m + (tok - tok)
        p = jnp.exp2(buf[c * CK:(c + 1) * CK, :].reshape(CK // 8, 8, TQ) - m8[None])
        cl = _tree(p, jnp.add) if 1 else jnp.sum(p, axis=0)
        toks.append(cl)
        o = jnp.dot(vt_sc[jnp.maximum(h, 0), :, c * CK:(c + 1) * CK], p.reshape(CK, TQ).astype(bf16), preferred_element_type=f32)
        if acc is None:
            return cl, o
        return acc[0] + cl, acc[1] + o

    def finalize(h, acc):
        l = jnp.sum(acc[0], axis=0, keepdims=True)
        ot_sc[pl.ds(pl.multiple_of((h + 1) * 16, 16), 16), :] = acc[1] / l

    def half(blk_q, h_q, wbuf, rbuf, tail, head):
        g, qm = qmask(blk_q, h_q)
        mx = None
        acc = None
        for c in range(NC):
            mx = qk_chunk(g, qm, c, wbuf, mx)
            if c < LAG:
                if tail is not None:
                    tail = (tail[0], tail[1], pv_chunk(tail[0], NC - LAG + c, wbuf, tail[1], tail[2]))
                    if c == LAG - 1:
                        finalize(tail[0], tail[2])
            elif head is not None:
                acc = pv_chunk(head[0], c - LAG, rbuf, head[1], acc)
        return jnp.max(mx, axis=0, keepdims=True), acc

    @pl.when(i == 0)
    def _prologue():
        cp_wmod_a().start()
        cp_x(0).start()
        cp_wqkv().start()
        cp_x(1).start()
        cp_wmod_b().start()
        cp_wo().start()
        cp_w1().start()
        cp_w2().start()
        c = jnp.broadcast_to(c_ref[...].astype(f32), (8, D))
        sc = (c * jax.nn.sigmoid(c)).astype(bf16)
        cp_wmod_a().wait()
        mod_sc[:, 0:2 * D] = jnp.dot(sc, wmod_v[:, 0:2 * D], preferred_element_type=f32)
        sa = mod_sc[0:1, 0:D]
        ca = mod_sc[0:1, D:2 * D]
        def qkv_chunk(r):
            rows = pl.ds(pl.multiple_of(r * TQ, TQ), TQ)
            xf = x_v[rows, :].astype(f32)
            h = _ln(xf) * (1.0 + ca) + sa
            qkv = jnp.dot(h.astype(bf16), wqkv_v[...], preferred_element_type=f32)
            kk = qkv[:, D:2 * D].astype(bf16)
            for g in range(4):
                k_sc[g, rows, :] = kk[:, g * 128:(g + 1) * 128]
            qt_sc[r] = (qkv[:, 0:D] * (DH ** -0.5 * LOG2E)).T.astype(bf16)
            vt = qkv[:, 2 * D:3 * D].T.astype(bf16)
            vt_sc[:, :, rows] = vt.reshape(H, DH, TQ)

        cp_x(0).wait()
        cp_wqkv().wait()
        qkv_chunk(0)
        cp_x(1).wait()
        PU = 2

        def qkv_body(j, carry):
            for u in range(PU):
                qkv_chunk(1 + j * PU + u)
            return carry

        nloop = (NQ - 1) // PU
        jax.lax.fori_loop(0, nloop, qkv_body, 0)
        for r in range(1 + nloop * PU, NQ):
            qkv_chunk(r)
        cp_wmod_b().wait()
        mod_sc[:, 2 * D:6 * D] = jnp.dot(sc, wmod_v[:, 2 * D:6 * D], preferred_element_type=f32)
        sb_sc[(NC - LAG) * CK:NC * CK, :] = jnp.zeros((LAG * CK, TQ), f32)
        m, _ = half(0, 0, sa_sc, None, None, None)
        m0_sc[...] = jnp.broadcast_to(m, (8, TQ))
        cp_wo().wait()
        cp_w1().wait()
        cp_w2().wait()

    toks.clear()
    m_0 = m0_sc[0:1, :]
    NH = 32

    def uhalf(hq, wbuf, rbuf, carry):
        m_p, la_p, oa_p, m_c = carry
        blk = jnp.minimum(i + hq // H, NQ - 1)
        m_n, acc_c = half(blk, hq % H, wbuf, rbuf, (hq - 2, m_p, (la_p, oa_p)), (hq - 1, m_c))
        return m_c, acc_c[0], acc_c[1], m_n

    def body(j, carry):
        toks.clear()
        for r in range(NH // 2):
            hq = j * NH + 2 * r + 1
            carry = uhalf(hq, sb_sc, sa_sc, carry)
            carry = uhalf(hq + 1, sa_sc, sb_sc, carry)
        return carry

    big = jnp.full((1, TQ), 3.0e38, f32)
    carry = (big, jnp.ones((8, TQ), f32), jnp.zeros((DH, TQ), f32), m_0)
    m_p, la_c, oa_c, m_n = jax.lax.fori_loop(0, H // NH, body, carry)
    toks.clear()
    m0_sc[...] = jnp.broadcast_to(m_n, (8, TQ))
    acc_c = (la_c, oa_c)
    for c in range(NC - LAG, NC):
        acc_c = pv_chunk(H - 1, c, sb_sc, m_p, acc_c)
    finalize(H - 1, acc_c)

    ga = mod_sc[0:1, 2 * D:3 * D]
    sb = mod_sc[0:1, 3 * D:4 * D]
    cb = mod_sc[0:1, 4 * D:5 * D]
    gb = mod_sc[0:1, 5 * D:6 * D]
    RS = 128
    nr = TQ // RS
    b1 = b1_ref[...].astype(f32).reshape(1, F)
    b2 = b2_ref[...].astype(f32).reshape(1, D)
    x1s = []
    for r in range(nr):
        o_att = ot_sc[16:16 + D, r * RS:(r + 1) * RS].T.astype(bf16)
        att = jnp.dot(o_att, wo_v[...], preferred_element_type=f32)
        rows = pl.ds(pl.multiple_of(i * TQ + r * RS, RS), RS)
        x1s.append(x_v[rows, :].astype(f32) + ga * att)
    us = []
    for r in range(nr):
        h2 = _ln(x1s[r]) * (1.0 + cb) + sb
        u = jnp.dot(h2.astype(bf16), w1_v[...], preferred_element_type=f32) + b1
        u = jnp.maximum(u, 0.0)
        us.append((u * u).astype(bf16))
    for r in range(nr):
        y = jnp.dot(us[r], w2_v[...], preferred_element_type=f32) + b2
        o_ref[r * RS:(r + 1) * RS, :] = (x1s[r] + gb * y).astype(o_ref.dtype)


@jax.jit
def pallas_adaLN_cond__mha_block__dense_activation_squared_relu__prompt_kernel(
    A_x, A_wqkv, A_wo, B_x, B_w1, B_b1, B_w2, B_b2, c, w_mod):
    del B_x
    x = A_x.reshape(S, D)
    full = lambda shape: pl.BlockSpec(shape, lambda i: (0,) * len(shape))
    hbm = pl.BlockSpec(memory_space=pl.ANY)
    out = pl.pallas_call(
        _kernel,
        grid=(NQ,),
        in_specs=[hbm, hbm, hbm, hbm, full((F,)), hbm, full((D,)), full((1, D)), hbm],
        out_specs=pl.BlockSpec((TQ, D), lambda i: (i, 0)),
        out_shape=jax.ShapeDtypeStruct((S, D), bf16),
        scratch_shapes=[
            pltpu.VMEM((S, D), bf16),
            pltpu.VMEM((D, 3 * D), bf16),
            pltpu.VMEM((D, D), bf16),
            pltpu.VMEM((D, F), bf16),
            pltpu.VMEM((F, D), bf16),
            pltpu.VMEM((D, 6 * D), bf16),
            pltpu.SemaphoreType.DMA((8,)),
            pltpu.VMEM((8, 6 * D), f32),
            pltpu.VMEM((4, S, 128), bf16),
            pltpu.VMEM((NQ, D, TQ), bf16),
            pltpu.VMEM((H, DH, S), bf16),
            pltpu.VMEM((D + 16, TQ), f32),
            pltpu.VMEM((S, TQ), f32),
            pltpu.VMEM((S, TQ), f32),
            pltpu.VMEM((8, TQ), f32),
        ],
        compiler_params=pltpu.CompilerParams(
            dimension_semantics=("arbitrary",),
            vmem_limit_bytes=100 * 1024 * 1024,
        ),
    )(x, A_wqkv, A_wo, B_w1, B_b1, B_w2, B_b2, c, w_mod)
    return out.reshape(1, S, D)
```

```python
import math
import jax
import jax.numpy as jnp
import jax.experimental.pallas as pl
import jax.experimental.pallas.tpu as pltpu

S = 2048
D = 512
H = 32
DH = 16
F = 1792
TQ = 256
NQ = S // TQ
CK = 128
NC = S // CK
LAG = 3
DEP = 1
EPS = 1e-5
LOG2E = math.log2(math.e)
f32 = jnp.float32
bf16 = jnp.bfloat16


def _ln(xf):
    mu = jnp.mean(xf, axis=-1, keepdims=True)
    xc = xf - mu
    var = jnp.mean(xc * xc, axis=-1, keepdims=True)
    return xc * jax.lax.rsqrt(var + EPS)


def _tree(x, op):
    parts = [x[j] for j in range(x.shape[0])]
    while len(parts) > 1:
        parts = [op(parts[j], parts[j + 1]) for j in range(0, len(parts) - 1, 2)] + (
            [parts[-1]] if len(parts) % 2 else [])
    return parts[0]


def _kernel(x_hbm, wqkv_hbm, wo_hbm, w1_hbm, b1_ref, w2_hbm, b2_ref, c_ref, wmod_hbm,
            o_ref,
            x_v, wqkv_v, wo_v, w1_v, w2_v, wmod_v, sems,
            mod_sc, k_sc, qt_sc, vt_sc, ot_sc, sa_sc, sb_sc, m0_sc, h_sc):
    i = pl.program_id(0)
    row128 = jax.lax.broadcasted_iota(jnp.int32, (128, TQ), 0)

    def cp_wmod_a():
        return pltpu.make_async_copy(wmod_hbm.at[:, pl.ds(0, 2 * D)], wmod_v.at[:, pl.ds(0, 2 * D)], sems.at[0])

    def cp_wmod_b():
        return pltpu.make_async_copy(wmod_hbm.at[:, pl.ds(2 * D, 4 * D)], wmod_v.at[:, pl.ds(2 * D, 4 * D)], sems.at[1])

    def cp_wqkv():
        return pltpu.make_async_copy(wqkv_hbm, wqkv_v, sems.at[2])

    def cp_wo():
        return pltpu.make_async_copy(wo_hbm, wo_v, sems.at[3])

    def cp_w1():
        return pltpu.make_async_copy(w1_hbm, w1_v, sems.at[4])

    def cp_w2():
        return pltpu.make_async_copy(w2_hbm, w2_v, sems.at[5])

    def cp_x(r):
        lo, n = (0, 3 * TQ) if r == 0 else (3 * TQ, S - 3 * TQ)
        return pltpu.make_async_copy(x_hbm.at[pl.ds(lo, n), :], x_v.at[pl.ds(lo, n), :], sems.at[6 + r])

    def qmask(blk, h):
        g = h // 8
        hh = h % 8
        qg = qt_sc[blk, pl.ds(pl.multiple_of(g * 128, 128), 128), :]
        return g, jnp.where((row128 >= hh * 16) & (row128 < hh * 16 + 16), qg, jnp.zeros_like(qg))

    def qk_chunk(g, qm, c, buf, mx):
        s = jnp.dot(k_sc[g, c * CK:(c + 1) * CK, :], qm, preferred_element_type=f32)
        buf[c * CK:(c + 1) * CK, :] = s
        cm = _tree(s.reshape(CK // 8, 8, TQ), jnp.maximum)
        return cm if mx is None else jnp.maximum(mx, cm)

    toks = []

    def pv_chunk(h, c, buf, m, acc):
        tok = toks[-DEP] if len(toks) >= DEP else None
        m8 = jnp.broadcast_to(m, (8, TQ)) if tok is None else m + (tok - tok)
        p = jnp.exp2(buf[c * CK:(c + 1) * CK, :].reshape(CK // 8, 8, TQ) - m8[None])
        cl = _tree(p, jnp.add)
        toks.append(cl)
        o = jnp.dot(vt_sc[jnp.maximum(h, 0), :, c * CK:(c + 1) * CK], p.reshape(CK, TQ).astype(bf16), preferred_element_type=f32)
        if acc is None:
            return cl, o
        return acc[0] + cl, acc[1] + o

    def finalize(h, acc):
        l = jnp.sum(acc[0], axis=0, keepdims=True)
        ot_sc[pl.ds(pl.multiple_of((h + 1) * 16, 16), 16), :] = acc[1] / l

    def half(blk_q, h_q, wbuf, rbuf, tail, head):
        g, qm = qmask(blk_q, h_q)
        mx = None
        acc = None
        for c in range(NC):
            mx = qk_chunk(g, qm, c, wbuf, mx)
            if c < LAG:
                if tail is not None:
                    tail = (tail[0], tail[1], pv_chunk(tail[0], NC - LAG + c, wbuf, tail[1], tail[2]))
                    if c == LAG - 1:
                        finalize(tail[0], tail[2])
            elif head is not None:
                acc = pv_chunk(head[0], c - LAG, rbuf, head[1], acc)
        return jnp.max(mx, axis=0, keepdims=True), acc

    @pl.when(i == 0)
    def _prologue():
        cp_wmod_a().start()
        cp_x(0).start()
        cp_wqkv().start()
        cp_x(1).start()
        cp_wmod_b().start()
        cp_wo().start()
        cp_w1().start()
        cp_w2().start()
        c = jnp.broadcast_to(c_ref[...].astype(f32), (8, D))
        sc = (c * jax.nn.sigmoid(c)).astype(bf16)
        cp_wmod_a().wait()
        mod_sc[:, 0:2 * D] = jnp.dot(sc, wmod_v[:, 0:2 * D], preferred_element_type=f32)
        sa = mod_sc[0:1, 0:D]
        ca = mod_sc[0:1, D:2 * D]

        def ln_chunk(r):
            rows = pl.ds(pl.multiple_of(r * TQ, TQ), TQ)
            h_sc[rows, :] = (_ln(x_v[rows, :].astype(f32)) * (1.0 + ca) + sa).astype(bf16)

        def qkv_chunk(r):
            rows = pl.ds(pl.multiple_of(r * TQ, TQ), TQ)
            qkv = jnp.dot(h_sc[rows, :], wqkv_v[...], preferred_element_type=f32)
            kk = qkv[:, D:2 * D].astype(bf16)
            for g in range(4):
                k_sc[g, rows, :] = kk[:, g * 128:(g + 1) * 128]
            qt_sc[r] = (qkv[:, 0:D] * (DH ** -0.5 * LOG2E)).T.astype(bf16)
            vt = qkv[:, 2 * D:3 * D].T.astype(bf16)
            vt_sc[:, :, rows] = vt.reshape(H, DH, TQ)

        cp_x(0).wait()
        ln_chunk(0)
        cp_wqkv().wait()
        qkv_chunk(0)
        ln_chunk(1)
        ln_chunk(2)
        cp_x(1).wait()

        def qkv_body(j, carry):
            qkv_chunk(1 + 2 * j)
            ln_chunk(3 + 2 * j)
            qkv_chunk(2 + 2 * j)
            ln_chunk(jnp.minimum(4 + 2 * j, NQ - 1))
            return carry

        jax.lax.fori_loop(0, 3, qkv_body, 0)
        qkv_chunk(NQ - 1)
        cp_wmod_b().wait()
        mod_sc[:, 2 * D:6 * D] = jnp.dot(sc, wmod_v[:, 2 * D:6 * D], preferred_element_type=f32)
        sb_sc[(NC - LAG) * CK:NC * CK, :] = jnp.zeros((LAG * CK, TQ), f32)
        m, _ = half(0, 0, sa_sc, None, None, None)
        m0_sc[...] = jnp.broadcast_to(m, (8, TQ))
        cp_wo().wait()
        cp_w1().wait()
        cp_w2().wait()

    toks.clear()
    m_0 = m0_sc[0:1, :]
    NH = 32

    def uhalf(hq, wbuf, rbuf, carry):
        m_p, la_p, oa_p, m_c = carry
        blk = jnp.minimum(i + hq // H, NQ - 1)
        m_n, acc_c = half(blk, hq % H, wbuf, rbuf, (hq - 2, m_p, (la_p, oa_p)), (hq - 1, m_c))
        return m_c, acc_c[0], acc_c[1], m_n

    def body(j, carry):
        toks.clear()
        for r in range(NH // 2):
            hq = j * NH + 2 * r + 1
            carry = uhalf(hq, sb_sc, sa_sc, carry)
            carry = uhalf(hq + 1, sa_sc, sb_sc, carry)
        return carry

    big = jnp.full((1, TQ), 3.0e38, f32)
    carry = (big, jnp.ones((8, TQ), f32), jnp.zeros((DH, TQ), f32), m_0)
    m_p, la_c, oa_c, m_n = jax.lax.fori_loop(0, H // NH, body, carry)
    toks.clear()
    m0_sc[...] = jnp.broadcast_to(m_n, (8, TQ))
    acc_c = (la_c, oa_c)
    for c in range(NC - LAG, NC):
        acc_c = pv_chunk(H - 1, c, sb_sc, m_p, acc_c)
    finalize(H - 1, acc_c)

    ga = mod_sc[0:1, 2 * D:3 * D]
    sb = mod_sc[0:1, 3 * D:4 * D]
    cb = mod_sc[0:1, 4 * D:5 * D]
    gb = mod_sc[0:1, 5 * D:6 * D]
    RS = 128
    nr = TQ // RS
    b1 = b1_ref[...].astype(f32).reshape(1, F)
    b2 = b2_ref[...].astype(f32).reshape(1, D)
    x1s = []
    for r in range(nr):
        o_att = ot_sc[16:16 + D, r * RS:(r + 1) * RS].T.astype(bf16)
        att = jnp.dot(o_att, wo_v[...], preferred_element_type=f32)
        rows = pl.ds(pl.multiple_of(i * TQ + r * RS, RS), RS)
        x1s.append(x_v[rows, :].astype(f32) + ga * att)
    us = []
    for r in range(nr):
        h2 = _ln(x1s[r]) * (1.0 + cb) + sb
        u = jnp.dot(h2.astype(bf16), w1_v[...], preferred_element_type=f32) + b1
        u = jnp.maximum(u, 0.0)
        us.append((u * u).astype(bf16))
    for r in range(nr):
        y = jnp.dot(us[r], w2_v[...], preferred_element_type=f32) + b2
        o_ref[r * RS:(r + 1) * RS, :] = (x1s[r] + gb * y).astype(o_ref.dtype)


@jax.jit
def pallas_adaLN_cond__mha_block__dense_activation_squared_relu__prompt_kernel(
    A_x, A_wqkv, A_wo, B_x, B_w1, B_b1, B_w2, B_b2, c, w_mod):
    del B_x
    x = A_x.reshape(S, D)
    full = lambda shape: pl.BlockSpec(shape, lambda i: (0,) * len(shape))
    hbm = pl.BlockSpec(memory_space=pl.ANY)
    out = pl.pallas_call(
        _kernel,
        grid=(NQ,),
        in_specs=[hbm, hbm, hbm, hbm, full((F,)), hbm, full((D,)), full((1, D)), hbm],
        out_specs=pl.BlockSpec((TQ, D), lambda i: (i, 0)),
        out_shape=jax.ShapeDtypeStruct((S, D), bf16),
        scratch_shapes=[
            pltpu.VMEM((S, D), bf16),
            pltpu.VMEM((D, 3 * D), bf16),
            pltpu.VMEM((D, D), bf16),
            pltpu.VMEM((D, F), bf16),
            pltpu.VMEM((F, D), bf16),
            pltpu.VMEM((D, 6 * D), bf16),
            pltpu.SemaphoreType.DMA((8,)),
            pltpu.VMEM((8, 6 * D), f32),
            pltpu.VMEM((4, S, 128), bf16),
            pltpu.VMEM((NQ, D, TQ), bf16),
            pltpu.VMEM((H, DH, S), bf16),
            pltpu.VMEM((D + 16, TQ), f32),
            pltpu.VMEM((S, TQ), f32),
            pltpu.VMEM((S, TQ), f32),
            pltpu.VMEM((8, TQ), f32),
            pltpu.VMEM((S, D), bf16),
        ],
        compiler_params=pltpu.CompilerParams(
            dimension_semantics=("arbitrary",),
            vmem_limit_bytes=100 * 1024 * 1024,
        ),
    )(x, A_wqkv, A_wo, B_w1, B_b1, B_w2, B_b2, c, w_mod)
    return out.reshape(1, S, D)
```
